```python
import jax
import jax.numpy as jnp

def _softmax(x, axis=-1):
    return jax.nn.softmax(x, axis=axis)
def _gelu(x):
    return jax.nn.gelu(x, approximate=True)
def _silu(x):
    return jax.nn.silu(x)
def _sigmoid(x):
    return jax.nn.sigmoid(x)
def _layernorm(x, axis=-1, eps=1e-5):
    m = jnp.mean(x, axis=axis, keepdims=True)
    v = jnp.var(x, axis=axis, keepdims=True)
    return (x - m) / jnp.sqrt(v + eps)
def _scatter_add(tgt, idx, src, axis=0):
    return tgt.at[idx].add(src)
def _segment_sum(src, seg, n):
    return jax.ops.segment_sum(src, seg, n)
class _Rng:
    def __init__(self, key):
        self._k = key
    def _next(self):
        self._k, sub = jax.random.split(self._k)
        return sub
    def normal(self, shape):
        return jax.random.normal(self._next(), shape, dtype=jnp.bfloat16)
    def randint(self, lo, hi, shape):
        return jax.random.randint(self._next(), shape, lo, hi, dtype=jnp.int32)
    def uniform(self, shape, lo=0.0, hi=1.0):
        return jax.random.uniform(self._next(), shape, jnp.bfloat16, lo, hi)
    def permutation(self, n):
        return jax.random.permutation(self._next(), n)


kernel_name = 'recurrent_scan__sliding_block_cached__moe_arch_mod__prompt'

def setup_inputs():
    _rng = _Rng(jax.random.key(int.from_bytes(__import__("os").urandom(4), "little")))
    _w = (lambda a: (lambda t: t.astype(jnp.bfloat16) if jnp.issubdtype(t.dtype, jnp.floating) else t)(jnp.asarray(a)))
    def _A_setup():
        B, Sq, D = 1, 2048, 640
        Hq, Hkv, Sk, Dh = 32, 32, 2048, 192
        assert Hq % Hkv == 0, (Hq, Hkv)
        return {
            "x": _w((lambda *s: _rng.normal(s) * 0.05)(B, Sq, D)),
            "k_cache": _w((lambda *s: _rng.normal(s) * 0.05)(B, Hkv, Sk, Dh)),
            "v_cache": _w((lambda *s: _rng.normal(s) * 0.05)(B, Hkv, Sk, Dh)),
            "wq": _w((lambda *s: _rng.normal(s) * 0.05)(D, Hq * Dh) * (D ** -0.5)),
            "wo": _w((lambda *s: _rng.normal(s) * 0.05)(Hq * Dh, D) * ((Hq * Dh) ** -0.5)),
        }
    _A_in = _A_setup()

    def _B_setup():
        B, S, D, F, C = 1, 2048, 640, 1536, 2
        return {
            "x": _w((lambda *s: _rng.normal(s) * 0.05)(B, S, D)),
            "w_r": _w((lambda *s: _rng.normal(s) * 0.05)(D)),
            "w_gate": _w((lambda *s: _rng.normal(s) * 0.05)(D, F)),
            "w_up": _w((lambda *s: _rng.normal(s) * 0.05)(D, F)),
            "w_down": _w((lambda *s: _rng.normal(s) * 0.05)(F, D)),
        }
    _B_in = _B_setup()

    return {
        "A_x": _A_in["x"],
        "A_k_cache": _A_in["k_cache"],
        "A_v_cache": _A_in["v_cache"],
        "A_wq": _A_in["wq"],
        "A_wo": _A_in["wo"],
        "B_x": _B_in["x"],
        "B_w_r": _B_in["w_r"],
        "B_w_gate": _B_in["w_gate"],
        "B_w_up": _B_in["w_up"],
        "B_w_down": _B_in["w_down"],
    }

def reference(A_x, A_k_cache, A_v_cache, A_wq, A_wo, B_x, B_w_r, B_w_gate, B_w_up, B_w_down):
    def _A_ref(x, k_cache, v_cache, wq, wo):
        B, Sq, D = x.shape
        Hq, Dh = 32, 192
        Hkv, Sk = k_cache.shape[1], k_cache.shape[2]
        W = min(4096, max(256, Sk // 4))
        rep = Hq // Hkv
        q = (lambda x, *d: x.transpose(*d))((x @ wq).reshape(B, Sq, Hq, Dh), 0, 2, 1, 3)
        k = jnp.repeat(k_cache[:, :, Sk - W:, :], rep, axis=1)
        v = jnp.repeat(v_cache[:, :, Sk - W:, :], rep, axis=1)
        scores = jnp.einsum("bhqd,bhkd->bhqk", q, k) * (Dh ** -0.5)
        p = _softmax(scores, axis=-1)
        o = jnp.einsum("bhqk,bhkd->bhqd", p, v)
        return (lambda x, *d: x.transpose(*d))(o, 0, 2, 1, 3).reshape(B, Sq, Hq * Dh) @ wo

    def _B_ref(x, w_r, w_gate, w_up, w_down):
        B, S, D = x.shape
        C = 2
        r = x @ w_r
        idx = jnp.argsort(-r, axis=-1)[:, :C]
        idx_e = jnp.repeat(idx.reshape(B, C, 1), D, axis=2)
        x_sel = jnp.take_along_axis(x, idx_e, axis=1)
        g = _silu(x_sel @ w_gate)
        u = x_sel @ w_up
        y = (g * u) @ w_down
        r_sel = _sigmoid(jnp.take_along_axis(r, idx, axis=1))
        y = y * r_sel.reshape(B, C, 1)
        b_off = (jnp.arange(B) * S).reshape(B, 1)
        flat_idx = (idx + b_off).reshape(B * C)
        zero = (x * 0.0).reshape(B * S, D)
        upd = _scatter_add(zero, flat_idx, y.reshape(B * C, D), axis=0)
        return x + upd.reshape(B, S, D)

    x = A_x
    xn = _layernorm(x, axis=-1)
    s = _A_ref(xn, A_k_cache, A_v_cache, A_wq, A_wo)
    g = _silu(_B_ref(xn, B_w_r, B_w_gate, B_w_up, B_w_down))
    return x + s * g
```

```python
import functools, os

import jax
import jax.numpy as jnp
import jax.experimental.pallas as pl
import jax.experimental.pallas.tpu as pltpu

F32 = jnp.float32
BF16 = jnp.bfloat16

S = 2048
D = 640
H = 32
DH = 192
SK = 2048
W = 512
FF = 1536
EPS = 1e-5

HP = 2
NP = H // HP
HD = HP * DH
CL = int(os.environ.get('CL', 512))
NCL = S // CL
CE = int(os.environ.get('CE', 512))
NCE = S // CE
ORDER = os.environ.get('ORDER', 'QSSOOP')
LG = int(os.environ.get('LG', 32))

SCALE_BF16 = 0.072265625
LOG2E = 1.4426950408889634
QSCALE = SCALE_BF16 * LOG2E


def _r(x):
    return x.astype(BF16).astype(F32)


def _sigmoid(x):
    return 0.5 * jnp.tanh(0.5 * x) + 0.5


def _silu(x):
    return x * _sigmoid(x)


def _dot(a, b):
    return jnp.dot(a, b, preferred_element_type=F32)


def _nt(a, b):
    return jax.lax.dot_general(a, b, (((1,), (1,)), ((), ())), preferred_element_type=F32)


def _kernel(x_hbm, kt_hbm, vt_hbm, wq_hbm, wo_hbm, wr_ref, wg_hbm, wu_hbm, wd_hbm,
            o_hbm,
            x_ref, xn_ref, q_ref, acc_ref, kt_ref, vt_ref, wq_ref, wo_ref,
            kpad_ref, wot_ref, ob_ref, wg_ref, wu_ref, wd_ref,
            xsem, ksem, vsem, qsem, psem, wsem, osem):

    def x_copy(c):
        rows = pl.ds(c * CL, CL)
        return pltpu.make_async_copy(x_hbm.at[rows, :], x_ref.at[rows, :], xsem.at[c])

    def _mul(p, n):
        return p * n if isinstance(p, int) else pl.multiple_of(p * n, n)

    def k_copy(p, slot):
        return pltpu.make_async_copy(
            kt_hbm.at[pl.ds(_mul(p, HP), HP), :, pl.ds(SK - W, W)], kt_ref.at[slot], ksem.at[slot])

    def v_copy(p, slot):
        return pltpu.make_async_copy(
            vt_hbm.at[pl.ds(_mul(p, HP), HP), :, pl.ds(SK - W, W)], vt_ref.at[slot], vsem.at[slot])

    def wq_copy(p, slot):
        return pltpu.make_async_copy(
            wq_hbm.at[:, pl.ds(_mul(p, HD), HD)], wq_ref.at[slot], qsem.at[slot])

    def wo_copy(p, slot):
        return pltpu.make_async_copy(
            wo_hbm.at[pl.ds(_mul(p, HD), HD), :], wo_ref.at[slot], psem.at[slot])

    def ffn_copies():
        return (pltpu.make_async_copy(wg_hbm, wg_ref, wsem.at[0]),
                pltpu.make_async_copy(wu_hbm, wu_ref, wsem.at[1]),
                pltpu.make_async_copy(wd_hbm, wd_ref, wsem.at[2]))

    def out_copy(c):
        rows = pl.ds(c * CE, CE)
        return pltpu.make_async_copy(ob_ref.at[rows, :], o_hbm.at[rows, :], osem.at[c])

    def prep(slot):
        zpad = jnp.zeros((256 - DH, W), BF16)
        kpad_ref[0] = jnp.concatenate([kt_ref[slot, 0], zpad], axis=0).T
        kpad_ref[1] = jnp.concatenate([zpad, kt_ref[slot, 1]], axis=0).T
        wot_ref[...] = wo_ref[slot].T

    def layernorm(c):
        for g in range(CL // LG):
            rows = pl.ds(c * CL + g * LG, LG)
            x = x_ref[rows, :].astype(F32)
            mu = jnp.sum(x, axis=-1, keepdims=True) * (1.0 / D)
            xc = x - mu
            var = jnp.sum(xc * xc, axis=-1, keepdims=True) * (1.0 / D)
            d = _r(x - _r(mu))
            ve = _r(_r(var) + EPS)
            sd = _r(ve * jax.lax.rsqrt(ve))
            inv = pl.reciprocal(sd, approx=True)
            inv = inv * (2.0 - sd * inv)
            xn_ref[rows, :] = (d * inv).astype(BF16)
        return xn_ref[pl.ds(c * CL, CL), :]

    def qproj(xn, slot):
        return (_dot(xn, wq_ref[slot]) * QSCALE).astype(BF16)

    def scores(h, slot):
        st = _nt(kpad_ref[h], q_ref[slot, :, 128 * h:128 * h + 256])
        m = jnp.max(st, axis=0, keepdims=True)
        e = jnp.exp2(st - m)
        l = jnp.sum(e, axis=0, keepdims=True)
        return e.astype(BF16), l

    def pv(pl_, h, slot):
        e, l = pl_
        ot = _dot(vt_ref[slot, h], e)
        return (ot * (1.0 / l)).astype(BF16)

    x_copy(0).start()
    wq_copy(0, 0).start()
    for c in range(1, NCL):
        x_copy(c).start()
    k_copy(0, 0).start()
    v_copy(0, 0).start()
    wo_copy(0, 0).start()
    wq_copy(1, 1).start()
    acc_ref[...] = jnp.zeros(acc_ref.shape, F32)
    x_copy(0).wait()
    layernorm(0)
    wq_copy(0, 0).wait()
    for c in range(NCL):
        if c + 1 < NCL:
            x_copy(c + 1).wait()
            layernorm(c + 1)
        q_ref[0, c * CL:(c + 1) * CL, :] = qproj(xn_ref[pl.ds(c * CL, CL), :], 0)

    def step_head(p, slot):
        k_copy(p, slot).wait()
        v_copy(p, slot).wait()
        wo_copy(p, slot).wait()

    def middle(p, carry):
        slot = p % 2
        nslot = 1 - slot
        step_head(p, slot)
        wq_copy(p + 1, nslot).wait()
        k_copy(p + 1, nslot).start()
        v_copy(p + 1, nslot).start()
        wo_copy(p + 1, nslot).start()

        @pl.when(p + 2 < NP)
        def _():
            wq_copy(p + 2, slot).start()

        @pl.when(p == 1)
        def _():
            for c in ffn_copies():
                c.start()

        prep(slot)

        env = {}
        for op in ORDER:
            if op == 'Q':
                q_ref[nslot] = qproj(xn_ref[...], nslot)
            elif op == 'S':
                h = len([k for k in env if k[0] == 'p'])
                env['p%d' % h] = scores(h, slot)
            elif op == 'O':
                h = len([k for k in env if k[0] == 'o'])
                env['o%d' % h] = pv(env['p%d' % h], h, slot)
            elif op == 'P':
                acc_ref[...] += _dot(wot_ref[...], jnp.concatenate([env['o0'], env['o1']], axis=0))
        return carry

    jax.lax.fori_loop(0, NP - 1, middle, 0)

    slot = (NP - 1) % 2
    step_head(NP - 1, slot)
    for c in ffn_copies():
        c.wait()
    prep(slot)

    wr = jnp.broadcast_to(wr_ref[...], (16, D))
    r = _r(_nt(wr, xn_ref[...])[0:1, :])
    ids = jax.lax.broadcasted_iota(jnp.int32, (1, S), 1)
    m0 = jnp.max(r, axis=1, keepdims=True)
    i0v = jnp.min(jnp.where(r == m0, ids, S - 1), axis=1, keepdims=True)
    r2 = jnp.where(ids == i0v, -jnp.inf, r)
    m1 = jnp.max(r2, axis=1, keepdims=True)
    i1v = jnp.min(jnp.where((r2 == m1) & (ids != i0v), ids, S - 1), axis=1, keepdims=True)
    i0 = i0v[0, 0]
    i1 = i1v[0, 0]
    sub = jax.lax.broadcasted_iota(jnp.int32, (16, D), 0)

    def group(i):
        base = pl.multiple_of(jnp.clip((i // 16) * 16, 0, S - 16), 16)
        return pl.ds(base, 16), sub == (i - base)

    rows0, hit0 = group(i0)
    rows1, hit1 = group(i1)
    x0 = jnp.sum(jnp.where(hit0, xn_ref[rows0, :].astype(F32), 0.0), axis=0, keepdims=True)
    x1 = jnp.sum(jnp.where(hit1, xn_ref[rows1, :].astype(F32), 0.0), axis=0, keepdims=True)
    xs = jnp.where(sub == 0, x0, jnp.where(sub == 1, x1, 0.0)).astype(BF16)

    p0 = scores(0, slot)
    gt = _r(_silu(_r(_dot(xs, wg_ref[...]))))
    up = _r(_dot(xs, wu_ref[...]))
    p1 = scores(1, slot)
    y = _r(_dot((gt * up).astype(BF16), wd_ref[...]))
    o0 = pv(p0, 0, slot)
    y0 = _r(y[0:1, :] * _r(_sigmoid(m0)))
    y1 = _r(y[1:2, :] * _r(_sigmoid(m1)))
    b0 = xn_ref[rows0, :].astype(F32)
    xn_ref[rows0, :] = jnp.where(hit0, b0 + y0, b0).astype(BF16)
    b1 = xn_ref[rows1, :].astype(F32)
    xn_ref[rows1, :] = jnp.where(hit1, b1 + y1, b1).astype(BF16)
    o1 = pv(p1, 1, slot)
    ot = jnp.concatenate([o0, o1], axis=0)

    for c in range(NCE):
        rows = pl.ds(c * CE, CE)
        st = acc_ref[:, c * CE:(c + 1) * CE] + _dot(wot_ref[...], ot[:, c * CE:(c + 1) * CE])
        g = _silu(xn_ref[rows, :].astype(F32))
        ob_ref[rows, :] = (x_ref[rows, :].astype(F32) + st.T * g).astype(BF16)
        out_copy(c).start()
    for c in range(NCE):
        out_copy(c).wait()


@jax.jit
def pallas_recurrent_scan__sliding_block_cached__moe_arch_mod__prompt_kernel(
    A_x: jax.Array,
    A_k_cache: jax.Array,
    A_v_cache: jax.Array,
    A_wq: jax.Array,
    A_wo: jax.Array,
    B_x: jax.Array,
    B_w_r: jax.Array,
    B_w_gate: jax.Array,
    B_w_up: jax.Array,
    B_w_down: jax.Array,
):
    x = A_x.reshape(S, D)
    kt = jnp.swapaxes(A_k_cache, 2, 3).reshape(H, DH, SK)
    vt = jnp.swapaxes(A_v_cache, 2, 3).reshape(H, DH, SK)
    wr = B_w_r.reshape(1, D)
    any_spec = pl.BlockSpec(memory_space=pl.ANY)
    dma = pltpu.SemaphoreType.DMA
    out = pl.pallas_call(
        _kernel,
        in_specs=[any_spec, any_spec, any_spec, any_spec, any_spec,
                  pl.BlockSpec(memory_space=pltpu.VMEM),
                  any_spec, any_spec, any_spec],
        out_specs=any_spec,
        out_shape=jax.ShapeDtypeStruct((S, D), BF16),
        scratch_shapes=[
            pltpu.VMEM((S, D), BF16),
            pltpu.VMEM((S, D), BF16),
            pltpu.VMEM((2, S, HD), BF16),
            pltpu.VMEM((D, S), F32),
            pltpu.VMEM((2, HP, DH, W), BF16),
            pltpu.VMEM((2, HP, DH, W), BF16),
            pltpu.VMEM((2, D, HD), BF16),
            pltpu.VMEM((2, HD, D), BF16),
            pltpu.VMEM((HP, W, 256), BF16),
            pltpu.VMEM((D, HD), BF16),
            pltpu.VMEM((S, D), BF16),
            pltpu.VMEM((D, FF), BF16),
            pltpu.VMEM((D, FF), BF16),
            pltpu.VMEM((FF, D), BF16),
            dma((NCL,)), dma((2,)), dma((2,)), dma((2,)), dma((2,)), dma((3,)), dma((NCE,)),
        ],
        compiler_params=pltpu.CompilerParams(
            vmem_limit_bytes=100 * 1024 * 1024,
        ),
    )(x, kt, vt, A_wq, A_wo, wr, B_w_gate, B_w_up, B_w_down)
    return out.reshape(1, S, D)
```

```python
import functools, os

import jax
import jax.numpy as jnp
import jax.experimental.pallas as pl
import jax.experimental.pallas.tpu as pltpu

F32 = jnp.float32
BF16 = jnp.bfloat16

S = 2048
D = 640
H = 32
DH = 192
SK = 2048
W = 512
FF = 1536
EPS = 1e-5

HP = 2
NP = H // HP
HD = HP * DH
XCH = [int(v) for v in os.environ.get('XCH', '256,256,512,512,512').split(',')]
XOFF = [sum(XCH[:i]) for i in range(len(XCH))]
NCL = len(XCH)
ECH = [int(v) for v in os.environ.get('ECH', '512,512,512,256,256').split(',')]
EOFF = [sum(ECH[:i]) for i in range(len(ECH))]
NCE = len(ECH)
ORDER = os.environ.get('ORDER', 'Q:0/4,S0,S1,Q:1/4,Q:2/4,Q:3/4,O0,O1,P')
LG = int(os.environ.get('LG', 32))
SC = 128

SCALE_BF16 = 0.072265625
LOG2E = 1.4426950408889634
QSCALE = SCALE_BF16 * LOG2E

L_LO = 2.0 ** -24
L_HI = 2.0 ** 40
F32_MAX = 3.0e38


def _r(x):
    return x.astype(BF16).astype(F32)


def _sigmoid(x):
    return 0.5 * jnp.tanh(0.5 * x) + 0.5


def _silu(x):
    return x * _sigmoid(x)


def _dot(a, b):
    return jnp.dot(a, b, preferred_element_type=F32)


def _nt(a, b):
    return jax.lax.dot_general(a, b, (((1,), (1,)), ((), ())), preferred_element_type=F32)


def _kernel(x_hbm, kt_hbm, vt_hbm, wq_hbm, wo_hbm, wr_hbm, wg_hbm, wu_hbm, wd_hbm,
            o_hbm,
            x_ref, xn_ref, q_ref, acc_ref, kt_ref, vt_ref, wq_ref, wo_ref,
            kpad_ref, wot_ref, bad_ref, ob_ref, wg_ref, wu_ref, wd_ref, wr_ref,
            xsem, ksem, vsem, qsem, psem, wsem, osem):

    def _mul(p, n):
        return p * n if isinstance(p, int) else pl.multiple_of(p * n, n)

    def x_copy(c):
        rows = pl.ds(XOFF[c], XCH[c])
        return pltpu.make_async_copy(x_hbm.at[rows, :], x_ref.at[rows, :], xsem.at[c])

    def k_copy(p, slot):
        return pltpu.make_async_copy(
            kt_hbm.at[pl.ds(_mul(p, HP), HP), :, pl.ds(SK - W, W)], kt_ref.at[slot], ksem.at[slot])

    def v_copy(p, slot):
        return pltpu.make_async_copy(
            vt_hbm.at[pl.ds(_mul(p, HP), HP), :, pl.ds(SK - W, W)], vt_ref.at[slot], vsem.at[slot])

    def wq_copy(p, slot):
        return pltpu.make_async_copy(
            wq_hbm.at[:, pl.ds(_mul(p, HD), HD)], wq_ref.at[slot], qsem.at[slot])

    def wo_copy(p, slot):
        return pltpu.make_async_copy(
            wo_hbm.at[pl.ds(_mul(p, HD), HD), :], wo_ref.at[slot], psem.at[slot])

    def ffn_copies():
        return (pltpu.make_async_copy(wg_hbm, wg_ref, wsem.at[0]),
                pltpu.make_async_copy(wu_hbm, wu_ref, wsem.at[1]),
                pltpu.make_async_copy(wd_hbm, wd_ref, wsem.at[2]),
                pltpu.make_async_copy(wr_hbm, wr_ref, wsem.at[3]))

    def out_copy(c):
        rows = pl.ds(EOFF[c], ECH[c])
        return pltpu.make_async_copy(ob_ref.at[rows, :], o_hbm.at[rows, :], osem.at[c])

    def prep(slot):
        zpad = jnp.zeros((256 - DH, W), BF16)
        kpad_ref[0] = jnp.concatenate([kt_ref[slot, 0], zpad], axis=0).T
        kpad_ref[1] = jnp.concatenate([zpad, kt_ref[slot, 1]], axis=0).T
        wot_ref[...] = wo_ref[slot].T

    def layernorm(r0, nrows):
        for g in range(nrows // LG):
            rows = pl.ds(r0 + g * LG, LG)
            x = x_ref[rows, :].astype(F32)
            mu = jnp.sum(x, axis=-1, keepdims=True) * (1.0 / D)
            mub = _r(mu)
            d = x - mub
            dm = mu - mub
            var = jnp.sum(d * d, axis=-1, keepdims=True) * (1.0 / D) - dm * dm
            ve = _r(_r(var) + EPS)
            sd = _r(ve * jax.lax.rsqrt(ve))
            inv = pl.reciprocal(sd, approx=True)
            inv = inv * (2.0 - sd * inv)
            xn_ref[rows, :] = (d * inv).astype(BF16)

    def qproj(xn, slot):
        return (_dot(xn, wq_ref[slot]) * QSCALE).astype(BF16)

    def scores(h, slot):
        st = _nt(kpad_ref[h], q_ref[slot, :, 128 * h:128 * h + 256])
        e = jnp.exp2(st)
        return e.astype(BF16), jnp.sum(e, axis=0, keepdims=True)

    def pv(sc, h, slot):
        e, l = sc
        o = _dot(vt_ref[slot, h], e) * (1.0 / l)
        omax = jnp.max(jnp.abs(o), axis=0, keepdims=True)
        ok = (l >= L_LO) & (l <= L_HI) & (omax <= F32_MAX)
        bad = jnp.where(ok, 0.0, 1.0)
        bad_ref[h] = bad
        return jnp.where(ok, o, 0.0).astype(BF16), jnp.max(bad, axis=1, keepdims=True)

    def exact_fallback(nbad, slot):
        @pl.when(nbad[0, 0] > 0.0)
        def _():
            def body(c, carry):
                cols = pl.ds(pl.multiple_of(c * SC, SC), SC)
                parts = []
                for h in range(HP):
                    st = _nt(kpad_ref[h], q_ref[slot, cols, 128 * h:128 * h + 256])
                    e = jnp.exp2(st - jnp.max(st, axis=0, keepdims=True))
                    l = jnp.sum(e, axis=0, keepdims=True)
                    ot = _dot(vt_ref[slot, h], e.astype(BF16))
                    parts.append(jnp.where(bad_ref[h, :, cols] > 0.0, ot * (1.0 / l), 0.0).astype(BF16))
                acc_ref[:, cols] += _dot(wot_ref[...], jnp.concatenate(parts, axis=0))
                return carry
            jax.lax.fori_loop(0, S // SC, body, 0)

    x_copy(0).start()
    wq_copy(0, 0).start()
    x_copy(1).start()
    acc_ref[...] = jnp.zeros(acc_ref.shape, F32)
    x_copy(0).wait()
    for c in range(2, NCL):
        x_copy(c).start()
    layernorm(XOFF[0], XCH[0])
    wq_copy(0, 0).wait()
    for c in range(NCL):
        if c + 1 < NCL:
            x_copy(c + 1).wait()
            if c == 0:
                k_copy(0, 0).start()
                v_copy(0, 0).start()
                wo_copy(0, 0).start()
                wq_copy(1, 1).start()
            layernorm(XOFF[c + 1], XCH[c + 1])
        rows = pl.ds(XOFF[c], XCH[c])
        q_ref[0, rows, :] = qproj(xn_ref[rows, :], 0)
    for c in ffn_copies():
        c.start()

    def step_head(p, slot):
        k_copy(p, slot).wait()
        v_copy(p, slot).wait()
        wo_copy(p, slot).wait()

    def middle(p, carry):
        slot = p % 2
        nslot = 1 - slot
        step_head(p, slot)
        wq_copy(p + 1, nslot).wait()
        k_copy(p + 1, nslot).start()
        v_copy(p + 1, nslot).start()
        wo_copy(p + 1, nslot).start()
        wq_copy(jnp.minimum(p + 2, NP - 1), slot).start()
        prep(slot)
        env = {}
        for tok in ORDER.split(','):
            op = tok[0]
            if ':' in tok:
                base, frac = tok.split(':')
                c, n = [int(v) for v in frac.split('/')]
            else:
                base, c, n = tok, 0, 1
            lo, hi = c * (S // n), (c + 1) * (S // n)
            if op == 'Q':
                q_ref[nslot, lo:hi, :] = qproj(xn_ref[lo:hi, :], nslot)
            elif op == 'S':
                h = int(base[1])
                env['s', h] = scores(h, slot)
            elif op == 'O':
                h = int(base[1])
                env['o', h] = pv(env['s', h], h, slot)
            elif op == 'P':
                ot = jnp.concatenate([env['o', 0][0], env['o', 1][0]], axis=0)
                acc_ref[:, lo:hi] += _dot(wot_ref[...], ot[:, lo:hi])
        exact_fallback(jnp.maximum(env['o', 0][1], env['o', 1][1]), slot)
        return carry

    jax.lax.fori_loop(0, NP - 1, middle, 0)
    wq_copy(NP - 1, (NP - 2) % 2).wait()

    slot = (NP - 1) % 2
    step_head(NP - 1, slot)
    for c in ffn_copies():
        c.wait()
    prep(slot)

    wr = wr_ref[...]
    r = None
    for k in range(D // 128):
        t = _nt(jnp.broadcast_to(wr[k:k + 1, :], (16, 128)), xn_ref[:, k * 128:(k + 1) * 128])
        r = t if r is None else r + t
    r = _r(r[0:1, :])
    ids = jax.lax.broadcasted_iota(jnp.int32, (1, S), 1)
    m0 = jnp.max(r, axis=1, keepdims=True)
    i0v = jnp.min(jnp.where(r == m0, ids, S - 1), axis=1, keepdims=True)
    r2 = jnp.where(ids == i0v, -jnp.inf, r)
    m1 = jnp.max(r2, axis=1, keepdims=True)
    i1v = jnp.min(jnp.where((r2 == m1) & (ids != i0v), ids, S - 1), axis=1, keepdims=True)
    i0 = i0v[0, 0]
    i1 = i1v[0, 0]
    sub = jax.lax.broadcasted_iota(jnp.int32, (16, D), 0)

    def group(i):
        base = pl.multiple_of(jnp.clip((i // 16) * 16, 0, S - 16), 16)
        return pl.ds(base, 16), sub == (i - base)

    rows0, hit0 = group(i0)
    rows1, hit1 = group(i1)
    x0 = jnp.sum(jnp.where(hit0, xn_ref[rows0, :].astype(F32), 0.0), axis=0, keepdims=True)
    x1 = jnp.sum(jnp.where(hit1, xn_ref[rows1, :].astype(F32), 0.0), axis=0, keepdims=True)
    xs = jnp.where(sub == 0, x0, jnp.where(sub == 1, x1, 0.0)).astype(BF16)

    s0 = scores(0, slot)
    gt = _r(_silu(_r(_dot(xs, wg_ref[...]))))
    up = _r(_dot(xs, wu_ref[...]))
    s1 = scores(1, slot)
    y = _r(_dot((gt * up).astype(BF16), wd_ref[...]))
    o0 = pv(s0, 0, slot)
    y0 = _r(y[0:1, :] * _r(_sigmoid(m0)))
    y1 = _r(y[1:2, :] * _r(_sigmoid(m1)))
    b0 = xn_ref[rows0, :].astype(F32)
    xn_ref[rows0, :] = jnp.where(hit0, b0 + y0, b0).astype(BF16)
    b1 = xn_ref[rows1, :].astype(F32)
    xn_ref[rows1, :] = jnp.where(hit1, b1 + y1, b1).astype(BF16)
    o1 = pv(s1, 1, slot)
    exact_fallback(jnp.maximum(o0[1], o1[1]), slot)
    ot = jnp.concatenate([o0[0], o1[0]], axis=0)

    for c in range(NCE):
        rows = pl.ds(EOFF[c], ECH[c])
        lo, hi = EOFF[c], EOFF[c] + ECH[c]
        st = acc_ref[:, lo:hi] + _dot(wot_ref[...], ot[:, lo:hi])
        g = _silu(xn_ref[rows, :].astype(F32))
        ob_ref[rows, :] = (x_ref[rows, :].astype(F32) + st.T * g).astype(BF16)
        out_copy(c).start()
    for c in range(NCE):
        out_copy(c).wait()


@jax.jit
def pallas_recurrent_scan__sliding_block_cached__moe_arch_mod__prompt_kernel(
    A_x: jax.Array,
    A_k_cache: jax.Array,
    A_v_cache: jax.Array,
    A_wq: jax.Array,
    A_wo: jax.Array,
    B_x: jax.Array,
    B_w_r: jax.Array,
    B_w_gate: jax.Array,
    B_w_up: jax.Array,
    B_w_down: jax.Array,
):
    x = A_x.reshape(S, D)
    kt = jnp.swapaxes(A_k_cache, 2, 3).reshape(H, DH, SK)
    vt = jnp.swapaxes(A_v_cache, 2, 3).reshape(H, DH, SK)
    wr = B_w_r.reshape(D // 128, 128)
    any_spec = pl.BlockSpec(memory_space=pl.ANY)
    dma = pltpu.SemaphoreType.DMA
    out = pl.pallas_call(
        _kernel,
        in_specs=[any_spec] * 9,
        out_specs=any_spec,
        out_shape=jax.ShapeDtypeStruct((S, D), BF16),
        scratch_shapes=[
            pltpu.VMEM((S, D), BF16),
            pltpu.VMEM((S, D), BF16),
            pltpu.VMEM((2, S, HD), BF16),
            pltpu.VMEM((D, S), F32),
            pltpu.VMEM((2, HP, DH, W), BF16),
            pltpu.VMEM((2, HP, DH, W), BF16),
            pltpu.VMEM((2, D, HD), BF16),
            pltpu.VMEM((2, HD, D), BF16),
            pltpu.VMEM((HP, W, 256), BF16),
            pltpu.VMEM((D, HD), BF16),
            pltpu.VMEM((HP, 1, S), F32),
            pltpu.VMEM((S, D), BF16),
            pltpu.VMEM((D, FF), BF16),
            pltpu.VMEM((D, FF), BF16),
            pltpu.VMEM((FF, D), BF16),
            pltpu.VMEM((D // 128, 128), BF16),
            dma((NCL,)), dma((2,)), dma((2,)), dma((2,)), dma((2,)), dma((4,)), dma((NCE,)),
        ],
        compiler_params=pltpu.CompilerParams(
            vmem_limit_bytes=100 * 1024 * 1024,
            disable_bounds_checks=True,
        ),
    )(x, kt, vt, A_wq, A_wo, wr, B_w_gate, B_w_up, B_w_down)
    return out.reshape(1, S, D)
```

```python
import functools, os

import jax
import jax.numpy as jnp
import jax.experimental.pallas as pl
import jax.experimental.pallas.tpu as pltpu

F32 = jnp.float32
BF16 = jnp.bfloat16

S = 2048
D = 640
H = 32
DH = 192
SK = 2048
W = 512
FF = 1536
EPS = 1e-5

HP = 2
NP = H // HP
HD = HP * DH
XCH = [int(v) for v in os.environ.get('XCH', '256,256,512,512,512').split(',')]
XOFF = [sum(XCH[:i]) for i in range(len(XCH))]
NCL = len(XCH)
ECH = [int(v) for v in os.environ.get('ECH', '512,512,512,256,256').split(',')]
EOFF = [sum(ECH[:i]) for i in range(len(ECH))]
NCE = len(ECH)
ORDER = os.environ.get('ORDER', 'Q:0/4,S0,S1,Q:1/4,Q:2/4,Q:3/4,O0,O1,P')
LG = int(os.environ.get('LG', 32))
RPOS = int(os.environ.get('RPOS', 0))
GU0 = int(os.environ.get('GU0', 2))
SC = 128

SCALE_BF16 = 0.072265625
LOG2E = 1.4426950408889634
QSCALE = SCALE_BF16 * LOG2E

L_LO = 2.0 ** -24
L_HI = 2.0 ** 40
F32_MAX = 3.0e38


def _r(x):
    return x.astype(BF16).astype(F32)


def _sigmoid(x):
    return 0.5 * jnp.tanh(0.5 * x) + 0.5


def _silu(x):
    return x * _sigmoid(x)


def _dot(a, b):
    return jnp.dot(a, b, preferred_element_type=F32)


def _nt(a, b):
    return jax.lax.dot_general(a, b, (((1,), (1,)), ((), ())), preferred_element_type=F32)


def _kernel(x_hbm, kt_hbm, vt_hbm, wq_hbm, wo_hbm, wr_hbm, wg_hbm, wu_hbm, wd_hbm,
            o_hbm,
            x_ref, xn_ref, q_ref, acc_ref, kt_ref, vt_ref, wq_ref, wo_ref,
            kpad_ref, wot_ref, bad_ref, ob_ref, wg_ref, wu_ref, wd_ref, wr_ref, r_ref,
            xsem, ksem, vsem, qsem, psem, wsem, osem):

    def _mul(p, n):
        return p * n if isinstance(p, int) else pl.multiple_of(p * n, n)

    def x_copy(c):
        rows = pl.ds(XOFF[c], XCH[c])
        return pltpu.make_async_copy(x_hbm.at[rows, :], x_ref.at[rows, :], xsem.at[c])

    def k_copy(p, slot):
        return pltpu.make_async_copy(
            kt_hbm.at[pl.ds(_mul(p, HP), HP), :, pl.ds(SK - W, W)], kt_ref.at[slot], ksem.at[slot])

    def v_copy(p, slot):
        return pltpu.make_async_copy(
            vt_hbm.at[pl.ds(_mul(p, HP), HP), :, pl.ds(SK - W, W)], vt_ref.at[slot], vsem.at[slot])

    def wq_copy(p, slot):
        return pltpu.make_async_copy(
            wq_hbm.at[:, pl.ds(_mul(p, HD), HD)], wq_ref.at[slot], qsem.at[slot])

    def wo_copy(p, slot):
        return pltpu.make_async_copy(
            wo_hbm.at[pl.ds(_mul(p, HD), HD), :], wo_ref.at[slot], psem.at[slot])

    def ffn_copies():
        return (pltpu.make_async_copy(wg_hbm, wg_ref, wsem.at[0]),
                pltpu.make_async_copy(wu_hbm, wu_ref, wsem.at[1]),
                pltpu.make_async_copy(wd_hbm, wd_ref, wsem.at[2]))

    def out_copy(c):
        rows = pl.ds(EOFF[c], ECH[c])
        return pltpu.make_async_copy(ob_ref.at[rows, :], o_hbm.at[rows, :], osem.at[c])

    def prep(slot):
        zpad = jnp.zeros((256 - DH, W), BF16)
        kpad_ref[0] = jnp.concatenate([kt_ref[slot, 0], zpad], axis=0).T
        kpad_ref[1] = jnp.concatenate([zpad, kt_ref[slot, 1]], axis=0).T
        wot_ref[...] = wo_ref[slot].T

    def layernorm(r0, nrows):
        for g in range(nrows // LG):
            rows = pl.ds(r0 + g * LG, LG)
            x = x_ref[rows, :].astype(F32)
            mu = jnp.sum(x, axis=-1, keepdims=True) * (1.0 / D)
            mub = _r(mu)
            d = x - mub
            dm = mu - mub
            var = jnp.sum(d * d, axis=-1, keepdims=True) * (1.0 / D) - dm * dm
            ve = _r(_r(var) + EPS)
            sd = _r(ve * jax.lax.rsqrt(ve))
            inv = pl.reciprocal(sd, approx=True)
            inv = inv * (2.0 - sd * inv)
            xn_ref[rows, :] = (d * inv).astype(BF16)

    def router(j):
        start = _mul(j, 128)
        xr = xn_ref[pl.ds(start, 128), :].astype(F32)
        wr = wr_ref[...].astype(F32)
        t = functools.reduce(jnp.add, [xr[:, k * 128:(k + 1) * 128] * wr[k:k + 1, :] for k in range(D // 128)])
        r_ref[:, pl.ds(start, 128)] = _r(jnp.sum(t.T, axis=0, keepdims=True))

    def qproj(xn, slot):
        return (_dot(xn, wq_ref[slot]) * QSCALE).astype(BF16)

    def scores(h, slot, lo=0, hi=S):
        st = _nt(kpad_ref[h], q_ref[slot, lo:hi, 128 * h:128 * h + 256])
        e = jnp.exp2(st)
        return e.astype(BF16), jnp.sum(e, axis=0, keepdims=True)

    def pv(sc, h, slot, lo=0, hi=S):
        e, l = sc
        o = _dot(vt_ref[slot, h], e) * (1.0 / l)
        omax = jnp.max(jnp.abs(o), axis=0, keepdims=True)
        ok = (l >= L_LO) & (l <= L_HI) & (omax <= F32_MAX)
        bad = jnp.where(ok, 0.0, 1.0)
        bad_ref[h, :, lo:hi] = bad
        return jnp.where(ok, o, 0.0).astype(BF16), jnp.max(bad, axis=1, keepdims=True)

    def exact_contrib(h, slot, cols, only_bad):
        lanes = pl.ds(pl.multiple_of(h * 128, 128), 256)
        st = _nt(kpad_ref[h], q_ref[slot, cols, lanes])
        e = jnp.exp2(st - jnp.max(st, axis=0, keepdims=True))
        l = jnp.sum(e, axis=0, keepdims=True)
        o = _dot(vt_ref[slot, h], e.astype(BF16)) * (1.0 / l)
        if only_bad:
            o = jnp.where(bad_ref[h, :, cols] > 0.0, o, 0.0)
        wo_h = wo_ref[slot, pl.ds(pl.multiple_of(h * DH, DH), DH), :]
        return jax.lax.dot_general(wo_h, o.astype(BF16), (((0,), (0,)), ((), ())),
                                   preferred_element_type=F32)

    def exact_fallback(nbad, slot):
        @pl.when(nbad[0, 0] > 0.0)
        def _():
            def body(i, carry):
                cols = pl.ds(pl.multiple_of((i // HP) * SC, SC), SC)
                acc_ref[:, cols] += exact_contrib(i % HP, slot, cols, True)
                return carry
            jax.lax.fori_loop(0, HP * (S // SC), body, 0)

    x_copy(0).start()
    wq_copy(0, 0).start()
    wr_copy = pltpu.make_async_copy(wr_hbm, wr_ref, wsem.at[3])
    wr_copy.start()
    x_copy(1).start()
    acc_ref[...] = jnp.zeros(acc_ref.shape, F32)
    x_copy(0).wait()
    for c in range(2, NCL):
        x_copy(c).start()
    layernorm(XOFF[0], XCH[0])
    wq_copy(0, 0).wait()
    wr_copy.wait()
    for c in range(NCL):
        if c + 1 < NCL:
            x_copy(c + 1).wait()
            if c == 0:
                k_copy(0, 0).start()
                v_copy(0, 0).start()
                wo_copy(0, 0).start()
                wq_copy(1, 1).start()
            layernorm(XOFF[c + 1], XCH[c + 1])
        rows = pl.ds(XOFF[c], XCH[c])
        q_ref[0, rows, :] = qproj(xn_ref[rows, :], 0)
    router(NP - 1)
    for c in ffn_copies():
        c.start()

    def step_head(p, slot):
        k_copy(p, slot).wait()
        v_copy(p, slot).wait()
        wo_copy(p, slot).wait()

    def middle(p, carry):
        slot = p % 2
        nslot = 1 - slot
        step_head(p, slot)
        wq_copy(p + 1, nslot).wait()
        k_copy(p + 1, nslot).start()
        v_copy(p + 1, nslot).start()
        wo_copy(p + 1, nslot).start()
        wq_copy(jnp.minimum(p + 2, NP - 1), slot).start()
        prep(slot)
        if RPOS == 0:
            router(p)
        env = {}
        toks = []
        for tok in ORDER.split(','):
            if '*' in tok:
                b, n = tok.split('*')
                toks += ['%s:%d/%s' % (b, i, n) for i in range(int(n))]
            else:
                toks.append(tok)
        for tok in toks:
            op = tok[0]
            if ':' in tok:
                base, frac = tok.split(':')
                c, n = [int(v) for v in frac.split('/')]
            else:
                base, c, n = tok, 0, 1
            lo, hi = c * (S // n), (c + 1) * (S // n)
            if op == 'Q':
                q_ref[nslot, lo:hi, :] = qproj(xn_ref[lo:hi, :], nslot)
            elif op == 'S':
                h = int(base[1])
                env['s', h, lo, hi] = scores(h, slot, lo, hi)
            elif op == 'O':
                h = int(base[1])
                ks = sorted([k for k in env if k[0] == 's' and k[1] == h and k[3] > lo and k[2] < hi], key=lambda k: k[2])
                es = [env[k][0][:, max(lo, k[2]) - k[2]:min(hi, k[3]) - k[2]] for k in ks]
                ls = [env[k][1][:, max(lo, k[2]) - k[2]:min(hi, k[3]) - k[2]] for k in ks]
                cat = lambda v: v[0] if len(v) == 1 else jnp.concatenate(v, axis=1)
                env['o', h, lo, hi] = pv((cat(es), cat(ls)), h, slot, lo, hi)
            elif op == 'P':
                parts = []
                for h in range(2):
                    ks = sorted([k for k in env if k[0] == 'o' and k[1] == h and k[3] > lo and k[2] < hi], key=lambda k: k[2])
                    cols = [env[k][0][:, max(lo, k[2]) - k[2]:min(hi, k[3]) - k[2]] for k in ks]
                    parts.append(cols[0] if len(cols) == 1 else jnp.concatenate(cols, axis=1))
                acc_ref[:, lo:hi] += _dot(wot_ref[...], jnp.concatenate(parts, axis=0))
        if RPOS == 1:
            router(p)
        exact_fallback(functools.reduce(jnp.maximum, [v[1] for k, v in env.items() if k[0] == 'o']), slot)
        return carry

    jax.lax.fori_loop(0, NP - 1, middle, 0)
    wq_copy(NP - 1, (NP - 2) % 2).wait()

    slot = (NP - 1) % 2
    step_head(NP - 1, slot)
    for c in ffn_copies():
        c.wait()
    prep(slot)

    r = r_ref[...]
    ids = jax.lax.broadcasted_iota(jnp.int32, (1, S), 1)
    m0 = jnp.max(r, axis=1, keepdims=True)
    i0v = jnp.min(jnp.where(r == m0, ids, S - 1), axis=1, keepdims=True)
    r2 = jnp.where(ids == i0v, -jnp.inf, r)
    m1 = jnp.max(r2, axis=1, keepdims=True)
    i1v = jnp.min(jnp.where((r2 == m1) & (ids != i0v), ids, S - 1), axis=1, keepdims=True)
    i0 = i0v[0, 0]
    i1 = i1v[0, 0]
    sub = jax.lax.broadcasted_iota(jnp.int32, (16, D), 0)

    def group(i):
        base = pl.multiple_of(jnp.clip((i // 16) * 16, 0, S - 16), 16)
        return pl.ds(base, 16), sub == (i - base)

    rows0, hit0 = group(i0)
    rows1, hit1 = group(i1)
    x0 = jnp.sum(jnp.where(hit0, xn_ref[rows0, :].astype(F32), 0.0), axis=0, keepdims=True)
    x1 = jnp.sum(jnp.where(hit1, xn_ref[rows1, :].astype(F32), 0.0), axis=0, keepdims=True)
    xs = jnp.where(sub == 0, x0, jnp.where(sub == 1, x1, 0.0)).astype(BF16)

    NG = 2 * FF // 512
    gu = [None] * NG

    def gu_piece(t):
        j, k = t // (D // 128), t % (D // 128)
        w_ref = wg_ref if j < NG // 2 else wu_ref
        c0 = (j % (NG // 2)) * 512
        v = _dot(xs[:, k * 128:(k + 1) * 128], w_ref[k * 128:(k + 1) * 128, c0:c0 + 512])
        gu[j] = v if gu[j] is None else gu[j] + v

    n_gu = NG * (D // 128)
    done = 0
    sc = {0: [], 1: []}
    for h in range(HP):
        for c in range(8):
            sc[h].append(scores(h, slot, c * 256, (c + 1) * 256))
            if (h * 8 + c >= GU0) and done < n_gu:
                gu_piece(done)
                done += 1

    def o_piece(h, c):
        e, l = sc[h][c // 2]
        half = (c % 2) * 128
        return pv((e[:, half:half + 128], l[:, half:half + 128]), h, slot, c * 128, (c + 1) * 128)

    o0 = []
    for c in range(16):
        o0.append(o_piece(0, c))
        if done < n_gu:
            gu_piece(done)
            done += 1
    while done < n_gu:
        gu_piece(done)
        done += 1
    gt = _r(_silu(_r(jnp.concatenate(gu[:NG // 2], axis=1))))
    up = _r(jnp.concatenate(gu[NG // 2:], axis=1))
    hid = (gt * up).astype(BF16)

    ylo = yhi = None
    o1 = []
    for c in range(16):
        o1.append(o_piece(1, c))
        if c < FF // 128:
            v = _dot(hid[:, c * 128:(c + 1) * 128], wd_ref[c * 128:(c + 1) * 128, 0:512])
            ylo = v if ylo is None else ylo + v
        elif c < FF // 128 + FF // 512:
            k = c - FF // 128
            v = _dot(hid[:, k * 512:(k + 1) * 512], wd_ref[k * 512:(k + 1) * 512, 512:D])
            yhi = v if yhi is None else yhi + v
    y = _r(jnp.concatenate([ylo, yhi], axis=1))
    y0 = _r(y[0:1, :] * _r(_sigmoid(m0)))
    y1 = _r(y[1:2, :] * _r(_sigmoid(m1)))
    b0 = xn_ref[rows0, :].astype(F32)
    xn_ref[rows0, :] = jnp.where(hit0, b0 + y0, b0).astype(BF16)
    b1 = xn_ref[rows1, :].astype(F32)
    xn_ref[rows1, :] = jnp.where(hit1, b1 + y1, b1).astype(BF16)
    nbad = functools.reduce(jnp.maximum, [o[1] for o in o0 + o1])
    ot = jnp.concatenate([jnp.concatenate([o[0] for o in o0], axis=1),
                          jnp.concatenate([o[0] for o in o1], axis=1)], axis=0)

    def finish(st, rows):
        g = _silu(xn_ref[rows, :].astype(F32))
        ob_ref[rows, :] = (x_ref[rows, :].astype(F32) + st.T * g).astype(BF16)

    for c in range(NCE):
        lo, hi = EOFF[c], EOFF[c] + ECH[c]
        finish(acc_ref[:, lo:hi] + _dot(wot_ref[...], ot[:, lo:hi]), pl.ds(EOFF[c], ECH[c]))
        out_copy(c).start()
    for c in range(NCE):
        out_copy(c).wait()

    @pl.when(nbad[0, 0] > 0.0)
    def _():
        def body(c, carry):
            cols = pl.ds(pl.multiple_of(c * SC, SC), SC)
            st = jax.lax.fori_loop(
                0, HP, lambda h, st: st + exact_contrib(h, slot, cols, False), acc_ref[:, cols])
            finish(st, cols)
            return carry
        jax.lax.fori_loop(0, S // SC, body, 0)
        for c in range(NCE):
            out_copy(c).start()
        for c in range(NCE):
            out_copy(c).wait()


@jax.jit
def pallas_recurrent_scan__sliding_block_cached__moe_arch_mod__prompt_kernel(
    A_x: jax.Array,
    A_k_cache: jax.Array,
    A_v_cache: jax.Array,
    A_wq: jax.Array,
    A_wo: jax.Array,
    B_x: jax.Array,
    B_w_r: jax.Array,
    B_w_gate: jax.Array,
    B_w_up: jax.Array,
    B_w_down: jax.Array,
):
    x = A_x.reshape(S, D)
    kt = jnp.swapaxes(A_k_cache, 2, 3).reshape(H, DH, SK)
    vt = jnp.swapaxes(A_v_cache, 2, 3).reshape(H, DH, SK)
    wr = B_w_r.reshape(D // 128, 128)
    any_spec = pl.BlockSpec(memory_space=pl.ANY)
    dma = pltpu.SemaphoreType.DMA
    out = pl.pallas_call(
        _kernel,
        in_specs=[any_spec] * 9,
        out_specs=any_spec,
        out_shape=jax.ShapeDtypeStruct((S, D), BF16),
        scratch_shapes=[
            pltpu.VMEM((S, D), BF16),
            pltpu.VMEM((S, D), BF16),
            pltpu.VMEM((2, S, HD), BF16),
            pltpu.VMEM((D, S), F32),
            pltpu.VMEM((2, HP, DH, W), BF16),
            pltpu.VMEM((2, HP, DH, W), BF16),
            pltpu.VMEM((2, D, HD), BF16),
            pltpu.VMEM((2, HD, D), BF16),
            pltpu.VMEM((HP, W, 256), BF16),
            pltpu.VMEM((D, HD), BF16),
            pltpu.VMEM((HP, 1, S), F32),
            pltpu.VMEM((S, D), BF16),
            pltpu.VMEM((D, FF), BF16),
            pltpu.VMEM((D, FF), BF16),
            pltpu.VMEM((FF, D), BF16),
            pltpu.VMEM((D // 128, 128), BF16),
            pltpu.VMEM((1, S), F32),
            dma((NCL,)), dma((2,)), dma((2,)), dma((2,)), dma((2,)), dma((4,)), dma((NCE,)),
        ],
        compiler_params=pltpu.CompilerParams(
            vmem_limit_bytes=100 * 1024 * 1024,
            disable_bounds_checks=True,
        ),
    )(x, kt, vt, A_wq, A_wo, wr, B_w_gate, B_w_up, B_w_down)
    return out.reshape(1, S, D)
```

```python
import functools

import jax
import jax.numpy as jnp
import jax.experimental.pallas as pl
import jax.experimental.pallas.tpu as pltpu

F32 = jnp.float32
BF16 = jnp.bfloat16

S = 2048
D = 640
H = 32
DH = 192
SK = 2048
W = 512
FF = 1536
EPS = 1.0013580322265625e-05

HP = 2
NP = H // HP
HD = HP * DH
LANE = 128
KPAD = 256

XCH = (256, 384, 640, 768)
XOFF = tuple(sum(XCH[:i]) for i in range(len(XCH)))
ECH = (512, 512, 512, 256, 256)
EOFF = tuple(sum(ECH[:i]) for i in range(len(ECH)))
SUB = 128
LG = 32
SC = 128
SQ = 256
OQ = 128
GU_START = 2

SCALE_BF16 = 0.072265625
LOG2E = 1.4426950408889634
QSCALE = SCALE_BF16 * LOG2E

L_LO = 2.0 ** -24
L_HI = 2.0 ** 40
F32_BIG = 3.0e38


def _r(x):
    return x.astype(BF16).astype(F32)


def _sigmoid(x):
    return 0.5 * jnp.tanh(0.5 * x) + 0.5


def _silu(x):
    return x * _sigmoid(x)


def _dot(a, b):
    return jnp.dot(a, b, preferred_element_type=F32)


def _nt(a, b):
    return jax.lax.dot_general(a, b, (((1,), (1,)), ((), ())), preferred_element_type=F32)


def _tn(a, b):
    return jax.lax.dot_general(a, b, (((0,), (0,)), ((), ())), preferred_element_type=F32)


def _mul(p, n):
    return p * n if isinstance(p, int) else pl.multiple_of(p * n, n)


def _kernel(x_hbm, kt_hbm, vt_hbm, wq_hbm, wo_hbm, wr_hbm, wg_hbm, wu_hbm, wd_hbm,
            o_hbm,
            x_ref, xn_ref, q_ref, acc_ref, kt_ref, vt_ref, wq_ref, wo_ref,
            kpad_ref, wot_ref, bad_ref, ob_ref, wg_ref, wu_ref, wd_ref, wr_ref, r_ref,
            xsem, ksem, vsem, qsem, psem, wsem, osem):

    def x_copy(c):
        rows = pl.ds(XOFF[c], XCH[c])
        return pltpu.make_async_copy(x_hbm.at[rows, :], x_ref.at[rows, :], xsem.at[c])

    def k_copy(p, slot):
        return pltpu.make_async_copy(
            kt_hbm.at[pl.ds(_mul(p, HP), HP), :, pl.ds(SK - W, W)], kt_ref.at[slot], ksem.at[slot])

    def v_copy(p, slot):
        return pltpu.make_async_copy(
            vt_hbm.at[pl.ds(_mul(p, HP), HP), :, pl.ds(SK - W, W)], vt_ref.at[slot], vsem.at[slot])

    def wq_copy(p, slot):
        return pltpu.make_async_copy(
            wq_hbm.at[:, pl.ds(_mul(p, HD), HD)], wq_ref.at[slot], qsem.at[slot])

    def wo_copy(p, slot):
        return pltpu.make_async_copy(
            wo_hbm.at[pl.ds(_mul(p, HD), HD), :], wo_ref.at[slot], psem.at[slot])

    def ffn_copies():
        return (pltpu.make_async_copy(wg_hbm, wg_ref, wsem.at[0]),
                pltpu.make_async_copy(wu_hbm, wu_ref, wsem.at[1]),
                pltpu.make_async_copy(wd_hbm, wd_ref, wsem.at[2]))

    def wr_copy():
        return pltpu.make_async_copy(wr_hbm, wr_ref, wsem.at[3])

    def out_copy(c):
        rows = pl.ds(EOFF[c], ECH[c])
        return pltpu.make_async_copy(ob_ref.at[rows, :], o_hbm.at[rows, :], osem.at[c])

    def prep(slot):
        zpad = jnp.zeros((KPAD - DH, W), BF16)
        kpad_ref[0] = jnp.concatenate([kt_ref[slot, 0], zpad], axis=0).T
        kpad_ref[1] = jnp.concatenate([zpad, kt_ref[slot, 1]], axis=0).T
        wot_ref[...] = wo_ref[slot].T

    def layernorm(r0, nrows):
        for g in range(nrows // LG):
            rows = pl.ds(r0 + g * LG, LG)
            x = x_ref[rows, :].astype(F32)
            mu = jnp.sum(x, axis=-1, keepdims=True) * (1.0 / D)
            mub = _r(mu)
            d = x - mub
            dm = mu - mub
            var = jnp.maximum(jnp.sum(d * d, axis=-1, keepdims=True) * (1.0 / D) - dm * dm, 0.0)
            ve = _r(_r(var) + EPS)
            sd = _r(ve * jax.lax.rsqrt(ve))
            inv = pl.reciprocal(sd, approx=True)
            inv = inv * (2.0 - sd * inv)
            xn_ref[rows, :] = (d * inv).astype(BF16)

    def router(j):
        start = _mul(j, LANE)
        xr = xn_ref[pl.ds(start, LANE), :].astype(F32)
        wr = wr_ref[...].astype(F32)
        t = functools.reduce(
            jnp.add, [xr[:, k * LANE:(k + 1) * LANE] * wr[k:k + 1, :] for k in range(D // LANE)])
        r_ref[:, pl.ds(start, LANE)] = _r(jnp.sum(t.T, axis=0, keepdims=True))

    def qproj(lo, hi, wslot, qslot):
        q = _dot(xn_ref[lo:hi, :], wq_ref[wslot]) * QSCALE
        q_ref[qslot, lo:hi, :] = q.astype(BF16)

    def scores(h, slot, lo, hi):
        st = _nt(kpad_ref[h], q_ref[slot, lo:hi, LANE * h:LANE * h + KPAD])
        e = jnp.exp2(st)
        return e.astype(BF16), jnp.sum(e, axis=0, keepdims=True)

    def pv(e, l, h, slot, lo, hi):
        o = _dot(vt_ref[slot, h], e) * (1.0 / l)
        omax = jnp.max(jnp.abs(o), axis=0, keepdims=True)
        ok = (l >= L_LO) & (l <= L_HI) & (omax <= F32_BIG)
        bad = jnp.where(ok, 0.0, 1.0)
        bad_ref[h, :, lo:hi] = bad
        return jnp.where(ok, o, 0.0).astype(BF16), jnp.max(bad, axis=1, keepdims=True)

    def pv_pieces(e, l, h, slot, between=None):
        outs = []
        for c in range(S // OQ):
            lo, hi = c * OQ, (c + 1) * OQ
            outs.append(pv(e[:, lo:hi], l[:, lo:hi], h, slot, lo, hi))
            if between is not None:
                between(c)
        return (jnp.concatenate([o[0] for o in outs], axis=1),
                functools.reduce(jnp.maximum, [o[1] for o in outs]))

    def exact_contrib(h, slot, cols, only_bad):
        lanes = pl.ds(pl.multiple_of(h * LANE, LANE), KPAD)
        st = _nt(kpad_ref[h], q_ref[slot, cols, lanes])
        e = jnp.exp2(st - jnp.max(st, axis=0, keepdims=True))
        l = jnp.sum(e, axis=0, keepdims=True)
        o = _dot(vt_ref[slot, h], e.astype(BF16)) * (1.0 / l)
        if only_bad:
            o = jnp.where(bad_ref[h, :, cols] > 0.0, o, 0.0)
        wo_h = wo_ref[slot, pl.ds(pl.multiple_of(h * DH, DH), DH), :]
        return _tn(wo_h, o.astype(BF16))

    x_copy(0).start()
    wq_copy(0, 0).start()
    wr_copy().start()
    x_copy(1).start()
    acc_ref[...] = jnp.zeros(acc_ref.shape, F32)
    x_copy(0).wait()
    for c in range(2, len(XCH)):
        x_copy(c).start()
    layernorm(0, SUB)
    wq_copy(0, 0).wait()
    wr_copy().wait()
    for j in range(S // SUB):
        nxt = (j + 1) * SUB
        if nxt < S:
            if nxt in XOFF:
                c = XOFF.index(nxt)
                x_copy(c).wait()
                if c == 1:
                    k_copy(0, 0).start()
                    v_copy(0, 0).start()
                    wo_copy(0, 0).start()
                    wq_copy(1, 1).start()
            layernorm(nxt, SUB)
        qproj(j * SUB, nxt, 0, 0)
    router(NP - 1)
    for cp in ffn_copies():
        cp.start()

    def step_wait(p, slot):
        k_copy(p, slot).wait()
        v_copy(p, slot).wait()
        wo_copy(p, slot).wait()

    def step(p, carry):
        slot = p % 2
        nslot = 1 - slot
        step_wait(p, slot)
        wq_copy(p + 1, nslot).wait()
        k_copy(p + 1, nslot).start()
        v_copy(p + 1, nslot).start()
        wo_copy(p + 1, nslot).start()
        wq_copy(jnp.minimum(p + 2, NP - 1), slot).start()
        prep(slot)
        router(p)
        qproj(0, S // 4, nslot, nslot)
        e0, l0 = scores(0, slot, 0, S)
        e1, l1 = scores(1, slot, 0, S)
        for c in range(1, 4):
            qproj(c * (S // 4), (c + 1) * (S // 4), nslot, nslot)
        o0, nbad0 = pv_pieces(e0, l0, 0, slot)
        o1, nbad1 = pv_pieces(e1, l1, 1, slot)
        acc_ref[...] += _dot(wot_ref[...], jnp.concatenate([o0, o1], axis=0))

        @pl.when(jnp.maximum(nbad0, nbad1)[0, 0] > 0.0)
        def _():
            def body(i, c2):
                cols = pl.ds(pl.multiple_of((i // HP) * SC, SC), SC)
                acc_ref[:, cols] += exact_contrib(i % HP, slot, cols, True)
                return c2
            jax.lax.fori_loop(0, HP * (S // SC), body, 0)

        return carry

    jax.lax.fori_loop(0, NP - 1, step, 0)
    wq_copy(NP - 1, (NP - 2) % 2).wait()

    slot = (NP - 1) % 2
    step_wait(NP - 1, slot)
    for cp in ffn_copies():
        cp.wait()
    prep(slot)

    r = r_ref[...]
    ids = jax.lax.broadcasted_iota(jnp.int32, (1, S), 1)
    m0 = jnp.max(r, axis=1, keepdims=True)
    i0v = jnp.min(jnp.where(r == m0, ids, S - 1), axis=1, keepdims=True)
    r2 = jnp.where(ids == i0v, -jnp.inf, r)
    m1 = jnp.max(r2, axis=1, keepdims=True)
    i1v = jnp.min(jnp.where((r2 == m1) & (ids != i0v), ids, S - 1), axis=1, keepdims=True)
    sub = jax.lax.broadcasted_iota(jnp.int32, (16, D), 0)

    def group(i):
        base = pl.multiple_of(jnp.clip((i // 16) * 16, 0, S - 16), 16)
        return pl.ds(base, 16), sub == (i - base)

    rows0, hit0 = group(i0v[0, 0])
    rows1, hit1 = group(i1v[0, 0])
    x0 = jnp.sum(jnp.where(hit0, xn_ref[rows0, :].astype(F32), 0.0), axis=0, keepdims=True)
    x1 = jnp.sum(jnp.where(hit1, xn_ref[rows1, :].astype(F32), 0.0), axis=0, keepdims=True)
    xs = jnp.where(sub == 0, x0, jnp.where(sub == 1, x1, 0.0)).astype(BF16)

    GW = 4 * LANE
    n_grp = 2 * FF // GW
    n_k = D // LANE
    gu = [None] * n_grp
    todo = list(range(n_grp * n_k))

    def gu_piece(_=None):
        if not todo:
            return
        t = todo.pop(0)
        j, k = t // n_k, t % n_k
        w_ref = wg_ref if j < n_grp // 2 else wu_ref
        c0 = (j % (n_grp // 2)) * GW
        v = _dot(xs[:, k * LANE:(k + 1) * LANE], w_ref[k * LANE:(k + 1) * LANE, c0:c0 + GW])
        gu[j] = v if gu[j] is None else gu[j] + v

    el = []
    for h in range(HP):
        parts = []
        for c in range(S // SQ):
            parts.append(scores(h, slot, c * SQ, (c + 1) * SQ))
            if h * (S // SQ) + c >= GU_START:
                gu_piece()
        el.append((jnp.concatenate([t[0] for t in parts], axis=1),
                   jnp.concatenate([t[1] for t in parts], axis=1)))
    o0, nbad0 = pv_pieces(el[0][0], el[0][1], 0, slot, gu_piece)
    while todo:
        gu_piece()
    gt = _r(_silu(_r(jnp.concatenate(gu[:n_grp // 2], axis=1))))
    up = _r(jnp.concatenate(gu[n_grp // 2:], axis=1))
    hid = (gt * up).astype(BF16)

    ys = {}

    def down_piece(c):
        if c < FF // LANE:
            key = 'lo'
            v = _dot(hid[:, c * LANE:(c + 1) * LANE], wd_ref[c * LANE:(c + 1) * LANE, 0:GW])
        elif c < FF // LANE + FF // GW:
            key, k = 'hi', c - FF // LANE
            v = _dot(hid[:, k * GW:(k + 1) * GW], wd_ref[k * GW:(k + 1) * GW, GW:D])
        else:
            return
        ys[key] = v if key not in ys else ys[key] + v

    o1, nbad1 = pv_pieces(el[1][0], el[1][1], 1, slot, down_piece)
    y = _r(jnp.concatenate([ys['lo'], ys['hi']], axis=1))
    y0 = _r(y[0:1, :] * _r(_sigmoid(m0)))
    y1 = _r(y[1:2, :] * _r(_sigmoid(m1)))
    b0 = xn_ref[rows0, :].astype(F32)
    xn_ref[rows0, :] = jnp.where(hit0, b0 + y0, b0).astype(BF16)
    b1 = xn_ref[rows1, :].astype(F32)
    xn_ref[rows1, :] = jnp.where(hit1, b1 + y1, b1).astype(BF16)
    ot = jnp.concatenate([o0, o1], axis=0)

    def finish(st, rows):
        g = _silu(xn_ref[rows, :].astype(F32))
        ob_ref[rows, :] = (x_ref[rows, :].astype(F32) + st.T * g).astype(BF16)

    for c in range(len(ECH)):
        lo, hi = EOFF[c], EOFF[c] + ECH[c]
        finish(acc_ref[:, lo:hi] + _dot(wot_ref[...], ot[:, lo:hi]), pl.ds(lo, ECH[c]))
        out_copy(c).start()
    for c in range(len(ECH)):
        out_copy(c).wait()

    @pl.when(jnp.maximum(nbad0, nbad1)[0, 0] > 0.0)
    def _():
        def body(c, carry):
            cols = pl.ds(pl.multiple_of(c * SC, SC), SC)
            st = jax.lax.fori_loop(
                0, HP, lambda h, a: a + exact_contrib(h, slot, cols, False), acc_ref[:, cols])
            finish(st, cols)
            return carry
        jax.lax.fori_loop(0, S // SC, body, 0)
        for c in range(len(ECH)):
            out_copy(c).start()
        for c in range(len(ECH)):
            out_copy(c).wait()


@jax.jit
def pallas_recurrent_scan__sliding_block_cached__moe_arch_mod__prompt_kernel(
    A_x: jax.Array,
    A_k_cache: jax.Array,
    A_v_cache: jax.Array,
    A_wq: jax.Array,
    A_wo: jax.Array,
    B_x: jax.Array,
    B_w_r: jax.Array,
    B_w_gate: jax.Array,
    B_w_up: jax.Array,
    B_w_down: jax.Array,
):
    del B_x
    x = A_x.reshape(S, D)
    kt = jnp.swapaxes(A_k_cache, 2, 3).reshape(H, DH, SK)
    vt = jnp.swapaxes(A_v_cache, 2, 3).reshape(H, DH, SK)
    wr = B_w_r.reshape(D // LANE, LANE)
    any_spec = pl.BlockSpec(memory_space=pl.ANY)
    dma = pltpu.SemaphoreType.DMA
    out = pl.pallas_call(
        _kernel,
        in_specs=[any_spec] * 9,
        out_specs=any_spec,
        out_shape=jax.ShapeDtypeStruct((S, D), BF16),
        scratch_shapes=[
            pltpu.VMEM((S, D), BF16),
            pltpu.VMEM((S, D), BF16),
            pltpu.VMEM((2, S, HD), BF16),
            pltpu.VMEM((D, S), F32),
            pltpu.VMEM((2, HP, DH, W), BF16),
            pltpu.VMEM((2, HP, DH, W), BF16),
            pltpu.VMEM((2, D, HD), BF16),
            pltpu.VMEM((2, HD, D), BF16),
            pltpu.VMEM((HP, W, KPAD), BF16),
            pltpu.VMEM((D, HD), BF16),
            pltpu.VMEM((HP, 1, S), F32),
            pltpu.VMEM((S, D), BF16),
            pltpu.VMEM((D, FF), BF16),
            pltpu.VMEM((D, FF), BF16),
            pltpu.VMEM((FF, D), BF16),
            pltpu.VMEM((D // LANE, LANE), BF16),
            pltpu.VMEM((1, S), F32),
            dma((len(XCH),)), dma((2,)), dma((2,)), dma((2,)), dma((2,)), dma((4,)),
            dma((len(ECH),)),
        ],
        compiler_params=pltpu.CompilerParams(
            vmem_limit_bytes=100 * 1024 * 1024,
            disable_bounds_checks=True,
        ),
    )(x, kt, vt, A_wq, A_wo, wr, B_w_gate, B_w_up, B_w_down)
    return out.reshape(1, S, D)
```
